```python
import os as _os
_os.environ.setdefault("JAX_PLATFORMS", "cpu")
import jax
import jax.numpy as jnp

def _softmax(x, axis=-1):
    return jax.nn.softmax(x, axis=axis)
def _gelu(x):
    return jax.nn.gelu(x, approximate=True)
def _silu(x):
    return jax.nn.silu(x)
def _sigmoid(x):
    return jax.nn.sigmoid(x)
def _layernorm(x, axis=-1, eps=1e-5):
    m = jnp.mean(x, axis=axis, keepdims=True)
    v = jnp.var(x, axis=axis, keepdims=True)
    return (x - m) / jnp.sqrt(v + eps)
def _scatter_add(tgt, idx, src, axis=0):
    return tgt.at[idx].add(src)
def _segment_sum(src, seg, n):
    return jax.ops.segment_sum(src, seg, n)
class _Rng:
    def __init__(self, key):
        self._k = key
    def _next(self):
        self._k, sub = jax.random.split(self._k)
        return sub
    def normal(self, shape):
        return jax.random.normal(self._next(), shape, dtype=jnp.bfloat16)
    def randint(self, lo, hi, shape):
        return jax.random.randint(self._next(), shape, lo, hi, dtype=jnp.int32)
    def uniform(self, shape, lo=0.0, hi=1.0):
        return jax.random.uniform(self._next(), shape, jnp.bfloat16, lo, hi)
    def permutation(self, n):
        return jax.random.permutation(self._next(), n)


kernel_name = 'standalone__mha_softmax__prompt'

def setup_inputs():
    _rng = _Rng(jax.random.key(int.from_bytes(__import__("os").urandom(4), "little")))
    _w = (lambda a: (lambda t: t.astype(jnp.bfloat16) if jnp.issubdtype(t.dtype, jnp.floating) else t)(jnp.asarray(a)))
    B, H, Sq, Sk, D = 1, 32, 2048, 2048, 192
    return {
        "q": _w((lambda *s: _rng.normal(s) * 0.4)(B, H, Sq, D)),
        "k": _w((lambda *s: _rng.normal(s) * 0.4)(B, H, Sk, D)),
        "v": _w((lambda *s: _rng.normal(s) * 0.05)(B, H, Sk, D)),
    }

def reference(q, k, v):
    scale = q.shape[-1] ** -0.5
    scores = jnp.einsum("bhqd,bhkd->bhqk", q, k) * scale
    p = _softmax(scores, axis=-1)
    return jnp.einsum("bhqk,bhkd->bhqd", p, v)
```

```python
import math

import numpy as np
import jax
import jax.numpy as jnp
import jax.experimental.pallas as pl
import jax.experimental.pallas.tpu as pltpu

f32 = jnp.float32
bf16 = jnp.bfloat16

TQ = 512
TK = 512


def _kernel(qt_ref, kt_ref, vt_ref, ot_ref, k_scr, s_scr, m_scr):
    D, S = kt_ref.shape
    tq, tk = TQ, TK
    nq = S // tq
    nc = S // tk
    hk = tk // 2
    c = float(np.asarray(D ** -0.5, dtype=bf16)) * math.log2(math.e)
    g = pl.program_id(0)
    ng = pl.num_programs(0)

    def prep(ci):
        kt = kt_ref[:, ci * tk:(ci + 1) * tk]
        a = kt[:, :hk].astype(f32)
        b = kt[:, hk:].astype(f32)
        l1 = jnp.concatenate([a[0:64] - b[0:64], a[64:128]], axis=0)
        l2 = jnp.concatenate([b[64:128], b[128:192] - a[128:192]], axis=0)
        l3 = jnp.concatenate([b[0:64], a[128:192]], axis=0)
        k_scr[0, ci * hk:(ci + 1) * hk, :] = l1.T.astype(bf16)
        k_scr[1, ci * hk:(ci + 1) * hk, :] = l2.T.astype(bf16)
        k_scr[2, ci * hk:(ci + 1) * hk, :] = l3.T.astype(bf16)

    def qk(ci, w):
        r = slice(ci * hk, (ci + 1) * hk)
        p3 = jnp.dot(k_scr[2, r, :], w[2], preferred_element_type=f32)
        p1 = jnp.dot(k_scr[0, r, :], w[0], preferred_element_type=f32)
        p2 = jnp.dot(k_scr[1, r, :], w[1], preferred_element_type=f32)
        return jnp.concatenate([p1 + p3, p2 + p3], axis=0)

    def weights(qi):
        qt = qt_ref[:, qi * tq:(qi + 1) * tq]
        return (qt[0:128], qt[64:192], jnp.concatenate([qt[0:64], qt[128:192]], axis=0))

    def red(x, op):
        return op(x.reshape(x.shape[0] // 8, 8, x.shape[1]), axis=0)

    def body(do1, do2):
        for qi in range(nq):
            cols = slice(qi * tq, (qi + 1) * tq)
            if do1:
                w = weights(qi)
            if do2:
                m_cur = m_scr[:, cols]
            m = None
            l = None
            acc = None
            for ci in range(nc):
                r = slice(ci * tk, (ci + 1) * tk)
                if do1 and qi == 0:
                    prep(ci)
                if do2:
                    p = jnp.exp2((s_scr[r, cols] - m_cur) * c)
                    ll = red(p, jnp.sum)
                    l = ll if l is None else l + ll
                    pb = p.astype(bf16)
                if do1:
                    s = qk(ci, w)
                    s_scr[r, cols] = s
                    mm = red(s, jnp.max)
                    m = mm if m is None else jnp.maximum(m, mm)
                if do2:
                    o = jnp.dot(vt_ref[:, r], pb, preferred_element_type=f32)
                    acc = o if acc is None else acc + o
            if do2:
                l = jnp.sum(l, axis=0, keepdims=True)
                ot_ref[:, cols] = (acc * (1.0 / l)).astype(ot_ref.dtype)
            if do1:
                m_scr[:, cols] = jnp.max(m, axis=0, keepdims=True)

    @pl.when(g == 0)
    def _():
        body(True, False)

    @pl.when(jnp.logical_and(g > 0, g < ng - 1))
    def _():
        body(True, True)

    @pl.when(g == ng - 1)
    def _():
        body(False, True)


@jax.jit
def pallas_standalone__mha_softmax__prompt_kernel(q: jax.Array, k: jax.Array, v: jax.Array):
    B, H, S, D = q.shape
    N = B * H
    tr = lambda x: jnp.swapaxes(x, 2, 3).reshape(N, D, x.shape[2])
    cur = pl.BlockSpec((None, D, S), lambda g: (jnp.minimum(g, N - 1), 0, 0))
    prev = pl.BlockSpec((None, D, S), lambda g: (jnp.maximum(g - 1, 0), 0, 0))
    ot = pl.pallas_call(
        _kernel,
        grid=(N + 1,),
        in_specs=[cur, cur, prev],
        out_specs=prev,
        out_shape=jax.ShapeDtypeStruct((N, D, S), q.dtype),
        scratch_shapes=[
            pltpu.VMEM((3, S // 2, 128), bf16),
            pltpu.VMEM((S, S), f32),
            pltpu.VMEM((1, S), f32),
        ],
        compiler_params=pltpu.CompilerParams(
            dimension_semantics=("arbitrary",),
            vmem_limit_bytes=100 * 1024 * 1024,
        ),
        name="mha",
    )(tr(q), tr(k), tr(v))
    return jnp.swapaxes(ot.reshape(B, H, D, S), 2, 3)
```

```python
import math

import numpy as np
import jax
import jax.numpy as jnp
from jax import lax
import jax.experimental.pallas as pl
import jax.experimental.pallas.tpu as pltpu

f32 = jnp.float32
bf16 = jnp.bfloat16

TQ = 512
TK = 512
V, K, Q = 0, 1, 2


def _kernel(q_hbm, k_hbm, v_hbm, o_hbm, inbuf, obuf, k_scr, m_scr, s_scr, isem, osem, psem):
    N, D, S = q_hbm.shape
    tq, tk = TQ, TK
    nq, nc, hk, dc = S // tq, S // tk, tk // 2, D // 3
    U = nq * nc
    c = float(np.asarray(D ** -0.5, dtype=bf16)) * math.log2(math.e)

    def prep(kt_ref, ci):
        kt = kt_ref[:, ci * tk:(ci + 1) * tk]
        a = kt[:, :hk].astype(f32)
        b = kt[:, hk:].astype(f32)
        l1 = jnp.concatenate([a[:dc] - b[:dc], a[dc:2 * dc]], axis=0)
        l2 = jnp.concatenate([b[dc:2 * dc], b[2 * dc:] - a[2 * dc:]], axis=0)
        l3 = jnp.concatenate([b[:dc], a[2 * dc:]], axis=0)
        for j, x in enumerate((l1, l2, l3)):
            k_scr[j, ci * hk:(ci + 1) * hk, :] = x.T.astype(bf16)

    def colsum8(p):
        parts = []
        for t in range(p.shape[0] // 128):
            acc = None
            for i in reversed(range(8)):
                r0 = t * 128 + i * 16
                x = p[r0:r0 + 8] + p[r0 + 8:r0 + 16]
                acc = x if acc is None else acc + x
            parts.append(acc)
        while len(parts) > 1:
            parts = [parts[i] + parts[i + 1] for i in range(0, len(parts), 2)]
        return parts[0]

    class Phase1:
        def __init__(self, qt_ref):
            self.qt_ref = qt_ref
            self.blocks = {}

        def open(self, qi, m=None, n=0):
            qt = self.qt_ref[:, qi * tq:(qi + 1) * tq]
            w = (qt[:2 * dc], qt[dc:], jnp.concatenate([qt[:dc], qt[2 * dc:]], axis=0))
            self.blocks[qi] = [w, m, n]

        def run(self, u):
            qi, ci = divmod(u, nc)
            cols = slice(qi * tq, (qi + 1) * tq)
            if qi not in self.blocks:
                self.open(qi)
            st = self.blocks[qi]
            r = slice(ci * hk, (ci + 1) * hk)
            t1, t2, t3 = [jnp.dot(k_scr[j, r, :], st[0][j], preferred_element_type=f32)
                          for j in range(3)]
            s = jnp.concatenate([t1 + t3, t2 + t3], axis=0)
            s_scr[u] = s
            mm = jnp.max(s.reshape(tk // 8, 8, tq), axis=0)
            st[1] = mm if st[1] is None else jnp.maximum(st[1], mm)
            st[2] += 1
            if st[2] == nc:
                m = jnp.max(st[1], axis=0, keepdims=True)
                m_scr[0, :, cols] = jnp.broadcast_to(m, (8, tq))
            elif u == U - 2:
                m_scr[1, :, cols] = st[1]
            return mm[0:1]

    def start_group(gv, gk, slot):
        pltpu.make_async_copy(v_hbm.at[gv], inbuf.at[slot, V], isem).start()
        pltpu.make_async_copy(k_hbm.at[gk], inbuf.at[slot, K], isem).start()
        pltpu.make_async_copy(q_hbm.at[gk], inbuf.at[slot, Q], isem).start()

    def wait_group(slot):
        pltpu.make_async_copy(inbuf.at[slot], inbuf.at[slot], isem).wait()

    def out_copy(h, slot):
        return pltpu.make_async_copy(obuf.at[slot], o_hbm.at[h], osem)

    def cols_copy(src, dst, lo, hi, i):
        return pltpu.make_async_copy(src.at[:, lo:hi], dst.at[:, lo:hi], psem.at[i])

    k0 = inbuf.at[2, K]
    q0 = inbuf.at[2, Q]
    kc = lambda lo, hi, i: cols_copy(k_hbm.at[0], k0, lo * tk, hi * tk, i)
    qc = lambda lo, hi, i: cols_copy(q_hbm.at[0], q0, lo * tq, hi * tq, i)
    cps = [kc(0, 1, 0), qc(0, 1, 1), qc(1, 2, 2), kc(1, 2, 3), kc(2, nc, 4), qc(2, nq, 5)]
    for d in cps:
        d.start()
    start_group(0, 1, 0)
    p1 = Phase1(q0)
    cps[0].wait()
    prep(k0, 0)
    cps[1].wait()
    p1.run(0)
    cps[2].wait()
    cps[3].wait()
    p1.run(nc)
    prep(k0, 1)
    p1.run(1)
    cps[4].wait()
    cps[5].wait()
    p1.run(nc + 1)
    for u in range(2, U - 1):
        if u in (nc, nc + 1):
            continue
        if u < nc:
            prep(k0, u)
        p1.run(u)

    def step(g, slot, pslot, oslot, last, never, start_dmas):
        vt_ref = inbuf.at[slot, V]
        ot_ref = obuf.at[oslot]
        tail = Phase1(inbuf.at[pslot, Q])
        tail.open(nq - 1, m_scr[1, :, (nq - 1) * tq:], nc - 1)
        start_dmas()
        p1 = Phase1(inbuf.at[slot, Q])
        outs = []
        marks = {}
        for t in range(U):
            qi, ci = divmod(t, nc)
            cols = slice(qi * tq, (qi + 1) * tq)
            if ci == 0:
                m, l, acc = m_scr[0, 0:1, cols], None, None
            m_t = m
            if qi == nq - 1:
                m_t = jnp.where(never, marks[t - (4 if last else 3)], m)
            p = jnp.exp2((s_scr[t] - m_t) * c)
            ll = colsum8(p)
            l = ll if l is None else l + ll
            o = jnp.dot(vt_ref[:, ci * tk:(ci + 1) * tk], p.astype(bf16),
                        preferred_element_type=f32)
            acc = o if acc is None else acc + o
            if last:
                marks[t] = o[0:1]
            if t == 0:
                tail.run(U - 1)
            elif not last:
                if t - 1 < nc:
                    prep(inbuf.at[slot, K], t - 1)
                marks[t] = p1.run(t - 1)
            if ci == nc - 1:
                l = jnp.sum(l, axis=0, keepdims=True)
                ot_ref[:, cols] = (acc * (1.0 / l)).astype(ot_ref.dtype)
                if last:
                    ns = 2 if qi == nq - 1 else 1
                    for j in range(ns):
                        lo = qi * tq + j * (tq // ns)
                        d = cols_copy(ot_ref, o_hbm.at[g], lo, lo + tq // ns, len(outs))
                        d.start()
                        outs.append(d)
        for d in outs:
            d.wait()

    def body(g, carry):
        slot, pslot, oslot = carry
        nslot = 3 - slot - pslot
        wait_group(slot)

        @pl.when(g >= 2)
        def _():
            out_copy(g - 2, oslot).wait()

        def start_dmas():
            @pl.when(g >= 1)
            def _():
                out_copy(g - 1, 1 - oslot).start()

            start_group(g + 1, jnp.minimum(g + 2, N - 1), nslot)

        step(g, slot, pslot, oslot, False, slot < 0, start_dmas)
        return nslot, slot, 1 - oslot

    fin = lax.fori_loop(0, N - 1, body, (jnp.int32(0), jnp.int32(2), jnp.int32(0)))
    gl = N - 1
    wait_group(gl % 3)
    out_copy(gl - 2, gl % 2).wait()
    step(gl, gl % 3, (gl - 1) % 3, gl % 2, True, fin[0] < 0,
         lambda: out_copy(gl - 1, (gl - 1) % 2).start())
    out_copy(gl - 1, (gl - 1) % 2).wait()


@jax.jit
def pallas_standalone__mha_softmax__prompt_kernel(q: jax.Array, k: jax.Array, v: jax.Array):
    B, H, S, D = q.shape
    N = B * H
    assert k.shape == q.shape and v.shape == q.shape
    assert D == 192 and S % TQ == 0 and S % TK == 0 and S // TQ >= 3 and S // TK >= 3 and N >= 3
    units = (S // TQ) * (S // TK)
    tr = lambda x: jnp.swapaxes(x, 2, 3).reshape(N, D, S)
    hbm = pl.BlockSpec(memory_space=pl.ANY)
    ot = pl.pallas_call(
        _kernel,
        in_specs=[hbm] * 3,
        out_specs=hbm,
        out_shape=jax.ShapeDtypeStruct((N, D, S), q.dtype),
        scratch_shapes=[
            pltpu.VMEM((3, 3, D, S), bf16),
            pltpu.VMEM((2, D, S), bf16),
            pltpu.VMEM((3, S // 2, 128), bf16),
            pltpu.VMEM((2, 8, S), f32),
            pltpu.VMEM((units, TK, TQ), f32),
            pltpu.SemaphoreType.DMA(()),
            pltpu.SemaphoreType.DMA(()),
            pltpu.SemaphoreType.DMA((max(6, S // TQ + 1),)),
        ],
        compiler_params=pltpu.CompilerParams(
            vmem_limit_bytes=100 * 1024 * 1024,
            disable_bounds_checks=True,
        ),
        name="mha",
    )(tr(q), tr(k), tr(v))
    return jnp.swapaxes(ot.reshape(B, H, D, S), 2, 3)
```

```python
import math

import numpy as np
import jax
import jax.numpy as jnp
from jax import lax
import jax.experimental.pallas as pl
import jax.experimental.pallas.tpu as pltpu

f32 = jnp.float32
bf16 = jnp.bfloat16

T = 128
W = 2 * T
GRP = 16
FIRST = 512
V, K, Q = 0, 1, 2


def _kernel(q_hbm, k_hbm, v_hbm, o_hbm, inbuf, obuf, k_scr, m_scr, g_scr, s_scr,
            isem, osem, psem):
    N, D, S = q_hbm.shape
    nb, hd, dc, ng = S // W, D // 2, D // 3, W // (8 * GRP)
    c = float(np.asarray(D ** -0.5, dtype=bf16)) * math.log2(math.e)
    units = [(qi, ci) for qi in range(nb) for ci in range(nb)]

    def prep(kt_ref, ci):
        kt = kt_ref[:, ci * W:(ci + 1) * W]
        a = kt[:, :T].astype(f32)
        b = kt[:, T:].astype(f32)
        l1 = jnp.concatenate([a[:dc] - b[:dc], a[dc:2 * dc]], axis=0)
        l2 = jnp.concatenate([b[dc:2 * dc], b[2 * dc:] - a[2 * dc:]], axis=0)
        l3 = jnp.concatenate([b[:dc], a[2 * dc:]], axis=0)
        for j, x in enumerate((l1, l2, l3)):
            k_scr[j, ci] = x.T.astype(bf16)

    def rowsum8(p):
        acc = None
        for i in reversed(range(T // 16)):
            x = p[i * 16:i * 16 + 8] + p[i * 16 + 8:i * 16 + 16]
            acc = x if acc is None else acc + x
        return acc

    class Offset:
        def __init__(self, qi, m, ga, n):
            self.qi, self.m, self.ga, self.n = qi, m, ga, n
            self.i, self.pos, self.e = 0, 0, None

        def advance(self, never=None, mark=None):
            self.i += 1
            end = (self.ga.shape[0] * self.i) // self.n
            m = self.m if mark is None else jnp.where(never, mark, self.m)
            e = jnp.sum(jnp.exp2((self.ga[self.pos:end] - m[None]) * (2 * c)), axis=0)
            self.e = e if self.e is None else self.e + e
            self.pos = end
            if self.i == self.n:
                e = jnp.sum(self.e, axis=0, keepdims=True)
                off = self.m + jnp.log2(e) * (0.5 / c)
                m_scr[0, :, self.qi * W:(self.qi + 1) * W] = jnp.broadcast_to(off, (8, W))
            return self.i == self.n

    class Phase1:
        def __init__(self, qt_ref, never, pending):
            self.qt_ref, self.never, self.pending = qt_ref, never, pending
            self.blocks = {}

        def begin(self, qi, m=None, gs=()):
            qt = self.qt_ref[:, qi * W:(qi + 1) * W]
            w = (qt[:2 * dc], qt[dc:], jnp.concatenate([qt[:dc], qt[2 * dc:]], axis=0))
            self.blocks[qi] = [w, m, list(gs)]

        def run(self, qi, ci, left=0):
            if qi not in self.blocks:
                self.begin(qi)
            st = self.blocks[qi]
            kl = [k_scr[j, ci] for j in range(3)]
            ts = [[None, None] for _ in range(3)]
            for h in range(2):
                for j in (2, 0, 1):
                    ts[j][h] = jnp.dot(kl[j], st[0][j][:, h * T:(h + 1) * T],
                                       preferred_element_type=f32)
            t1, t2, t3 = [jnp.concatenate(x, axis=1) for x in ts]
            s = jnp.concatenate([t1 + t3, t2 + t3], axis=0)
            s_scr[qi * nb + ci] = s
            gm = jnp.max(s.reshape(ng, GRP, 8, W), axis=1)
            mm = jnp.max(gm, axis=0)
            st[1] = mm if st[1] is None else jnp.maximum(st[1], mm)
            st[2].append(gm)
            if self.pending and self.pending[0].advance(self.never, mm[0:1]):
                self.pending.pop(0)
            if sum(x.shape[0] for x in st[2]) == nb * ng:
                m = jnp.max(st[1], axis=0, keepdims=True)
                ga = jnp.concatenate(st[2], axis=0)
                if self.never is None:
                    Offset(qi, m, ga, 1).advance()
                else:
                    self.pending.append(Offset(qi, m, ga, min(nb, left - 1)))
                del self.blocks[qi]
            return mm[0:1, :T]

        def save(self):
            (qi, st), = self.blocks.items()
            assert qi == nb - 1 and not self.pending
            m_scr[1, :, qi * W:] = st[1]
            g_scr[...] = jnp.concatenate(st[2], axis=0)

    def start_group(gv, gk, slot):
        pltpu.make_async_copy(v_hbm.at[gv], inbuf.at[slot, V], isem).start()
        pltpu.make_async_copy(k_hbm.at[gk], inbuf.at[slot, K], isem).start()
        pltpu.make_async_copy(q_hbm.at[gk], inbuf.at[slot, Q], isem).start()

    def wait_group(slot):
        pltpu.make_async_copy(inbuf.at[slot], inbuf.at[slot], isem).wait()

    def out_copy(h, slot):
        return pltpu.make_async_copy(obuf.at[slot], o_hbm.at[h], osem)

    def cols_copy(src, dst, lo, hi, i):
        return pltpu.make_async_copy(src.at[:, lo:hi], dst.at[:, lo:hi], psem.at[i])

    k0 = inbuf.at[2, K]
    q0 = inbuf.at[2, Q]
    F = FIRST
    cps = [cols_copy(k_hbm.at[0], k0, 0, F, 0), cols_copy(q_hbm.at[0], q0, 0, F, 1),
           cols_copy(q_hbm.at[0], q0, F, 2 * F, 2), cols_copy(k_hbm.at[0], k0, F, 2 * F, 3),
           cols_copy(k_hbm.at[0], k0, 2 * F, S, 4), cols_copy(q_hbm.at[0], q0, 2 * F, S, 5)]
    for d in cps:
        d.start()
    start_group(0, 1, 0)
    first = Phase1(q0, None, [])
    done, prepped = {units[-1]}, set()

    def rect(klo, khi, qlo, qhi):
        for qi in range(qlo // W, qhi // W):
            for ci in range(klo // W, khi // W):
                if (qi, ci) in done:
                    continue
                if ci not in prepped:
                    prep(k0, ci)
                    prepped.add(ci)
                first.run(qi, ci)
                done.add((qi, ci))

    cps[0].wait()
    for ci in range(F // W):
        prep(k0, ci)
        prepped.add(ci)
    cps[1].wait()
    rect(0, F, 0, F)
    cps[2].wait()
    cps[3].wait()
    rect(0, F, F, 2 * F)
    rect(F, 2 * F, 0, F)
    cps[4].wait()
    cps[5].wait()
    rect(F, 2 * F, F, 2 * F)
    rect(0, S, 0, S)
    first.save()

    def step(g, slot, pslot, oslot, last, never, start_dmas):
        vt_ref = inbuf.at[slot, V]
        ot_ref = obuf.at[oslot]
        pending = []
        tail = Phase1(inbuf.at[pslot, Q], None if last else never, pending)
        tail.begin(nb - 1, m_scr[1, :, (nb - 1) * W:], [g_scr[...]])
        start_dmas()
        nxt = Phase1(inbuf.at[slot, Q], never, pending)
        outs, marks, lhs = [], [], {}
        todo = [] if last else units[:-1]
        marks.append(tail.run(*units[-1], len(todo)))

        for t, (qi, ci) in enumerate(units):
            cols = slice(qi * W, (qi + 1) * W)
            if ci == 0:
                off, l, acc = m_scr[0, 0:1, cols], [None, None], [None] * 7
            if qi == 0:
                va = vt_ref[:, ci * W:ci * W + T]
                vb = vt_ref[:, ci * W + T:(ci + 1) * W]
                a11, a21, a12, a22 = va[:hd], va[hd:], vb[:hd], vb[hd:]
                add = lambda x, y: (x.astype(f32) + y.astype(f32)).astype(bf16)
                sub = lambda x, y: (x.astype(f32) - y.astype(f32)).astype(bf16)
                lhs[ci] = [add(a11, a22), add(a21, a22), a11, a22, add(a11, a12),
                           sub(a21, a11), sub(a12, a22)]

            def prob(k, q):
                o = off[:, q * T:(q + 1) * T]
                if qi == nb - 1:
                    o = jnp.where(never, marks[-(4 if last else 3)], o)
                p = jnp.exp2((s_scr[t, k * T:(k + 1) * T, q * T:(q + 1) * T] - o) * c)
                ll = rowsum8(p)
                l[q] = ll if l[q] is None else l[q] + ll
                return p

            b11, b22, b12, b21 = prob(0, 0), prob(1, 1), prob(0, 1), prob(1, 0)
            rhs = [b11 - b22, b11, b22 - b12, b21 - b11, b22, b11 - b12, b21 - b22]
            for i in range(7):
                o = jnp.dot(lhs[ci][i], rhs[i].astype(bf16), preferred_element_type=f32)
                acc[i] = o if acc[i] is None else acc[i] + o
            if last:
                marks.append(o[0:1])
            elif t > 0:
                if t - 1 < nb:
                    prep(inbuf.at[slot, K], t - 1)
                marks.append(nxt.run(*todo[t - 1], len(todo) - t))
            if ci == nb - 1:
                m1, m2, m3, m4, m5, m6, m7 = acc
                res = jnp.concatenate(
                    [jnp.concatenate([m1 + m4 + m5 + m7, m5 - m3], axis=1),
                     jnp.concatenate([m2 + m4, m2 - m1 - m3 - m6], axis=1)], axis=0)
                den = jnp.sum(jnp.concatenate(l, axis=1), axis=0, keepdims=True)
                ot_ref[:, cols] = (res * (1.0 / den)).astype(ot_ref.dtype)
                if last:
                    d = cols_copy(ot_ref, o_hbm.at[g], qi * W, (qi + 1) * W, qi)
                    d.start()
                    outs.append(d)
        if not last:
            nxt.save()
        for d in outs:
            d.wait()

    def body(g, carry):
        slot, pslot, oslot = carry
        nslot = 3 - slot - pslot
        wait_group(slot)

        @pl.when(g >= 2)
        def _():
            out_copy(g - 2, oslot).wait()

        def start_dmas():
            @pl.when(g >= 1)
            def _():
                out_copy(g - 1, 1 - oslot).start()

            start_group(g + 1, jnp.minimum(g + 2, N - 1), nslot)

        step(g, slot, pslot, oslot, False, slot < 0, start_dmas)
        return nslot, slot, 1 - oslot

    fin = lax.fori_loop(0, N - 1, body, (jnp.int32(0), jnp.int32(2), jnp.int32(0)))
    gl = N - 1
    wait_group(gl % 3)
    out_copy(gl - 2, gl % 2).wait()
    step(gl, gl % 3, (gl - 1) % 3, gl % 2, True, fin[0] < 0,
         lambda: out_copy(gl - 1, (gl - 1) % 2).start())
    out_copy(gl - 1, (gl - 1) % 2).wait()


@jax.jit
def pallas_standalone__mha_softmax__prompt_kernel(q: jax.Array, k: jax.Array, v: jax.Array):
    B, H, S, D = q.shape
    N = B * H
    assert k.shape == q.shape and v.shape == q.shape
    assert D == 192 and S % FIRST == 0 and S > 2 * FIRST and N >= 3
    nb = S // W
    tr = lambda x: jnp.swapaxes(x, 2, 3).reshape(N, D, S)
    hbm = pl.BlockSpec(memory_space=pl.ANY)
    ot = pl.pallas_call(
        _kernel,
        in_specs=[hbm] * 3,
        out_specs=hbm,
        out_shape=jax.ShapeDtypeStruct((N, D, S), q.dtype),
        scratch_shapes=[
            pltpu.VMEM((3, 3, D, S), bf16),
            pltpu.VMEM((2, D, S), bf16),
            pltpu.VMEM((3, nb, T, T), bf16),
            pltpu.VMEM((2, 8, S), f32),
            pltpu.VMEM(((nb - 1) * (W // (8 * GRP)), 8, W), f32),
            pltpu.VMEM((nb * nb, W, W), f32),
            pltpu.SemaphoreType.DMA(()),
            pltpu.SemaphoreType.DMA(()),
            pltpu.SemaphoreType.DMA((max(6, nb),)),
        ],
        compiler_params=pltpu.CompilerParams(
            vmem_limit_bytes=100 * 1024 * 1024,
            disable_bounds_checks=True,
        ),
        name="mha",
    )(tr(q), tr(k), tr(v))
    return jnp.swapaxes(ot.reshape(B, H, D, S), 2, 3)
```

```python
import functools
import math

import numpy as np
import jax
import jax.numpy as jnp
from jax import lax
import jax.experimental.pallas as pl
import jax.experimental.pallas.tpu as pltpu

f32 = jnp.float32
bf16 = jnp.bfloat16
u32 = jnp.uint32

T = 128
W = 2 * T
NT = 4
R = NT * T // W
LAM = (-1.5, -0.5, 0.5, 1.5)
NEG = ((0, 3), (1, 2))
JOBS = ((0, 1), (0, 2), (0, 3), (0,), (1, 2), (1, 3), (1,), (2, 3), (2,), (3,))
BASE = [int(x) for x in np.cumsum([0] + [len(j) + 1 for j in JOBS])]
NP = BASE[-1]
GRP = 16
TAIL = R * R
FIRST = 512
RATE = 34
V, K, Q = 0, 1, 2


def _sign(i, j):
    return -1 if (min(i, j), max(i, j)) in NEG else 1


def _addsub(x, y, s):
    return x + y if s > 0 else x - y


def _kernel(q_hbm, k_hbm, v_hbm, o_hbm, inbuf, obuf, k_scr, m_scr, g_scr, s_scr, a_scr, l_scr,
            va_scr, vb_scr, isem, osem, psem):
    N, D, S = q_hbm.shape
    nb, ns, hd, dc, ng = S // W, S // (NT * T), D // 2, D // 3, W // (8 * GRP)
    c = float(np.asarray(D ** -0.5, dtype=bf16)) * math.log2(math.e)
    enc = lambda x: pltpu.bitcast(x.astype(bf16), u32)
    dec = lambda x: pltpu.bitcast(x, bf16)
    units = [(Qs * R + a, Ks * R + b) for Qs in range(ns) for Ks in range(ns)
             for a in range(R) for b in range(R)]
    tail_units = units[-TAIL:]
    ntail = TAIL // R

    never = lax.fori_loop(0, 2, lambda i, x: 1 - x, jnp.int32(0)) < 0

    def gate(x, mark):
        if mark is None:
            return x
        return jnp.where(never, jnp.tile(mark[:x.shape[0]], (1, x.shape[1] // T)), x)

    def kprep(kt_ref, ci):
        kt = kt_ref[:, ci * W:(ci + 1) * W]
        a = kt[:, :T].astype(f32)
        b = kt[:, T:].astype(f32)
        l1 = jnp.concatenate([a[:dc] - b[:dc], a[dc:2 * dc]], axis=0)
        l2 = jnp.concatenate([b[dc:2 * dc], b[2 * dc:] - a[2 * dc:]], axis=0)
        l3 = jnp.concatenate([b[:dc], a[2 * dc:]], axis=0)
        for j, x in enumerate((l1, l2, l3)):
            k_scr[j, ci] = enc(x.T)

    def vprep(vt_ref, Ks, b):
        job = JOBS[b]
        nr = 16 if len(job) == 2 else 32

        def piece(r0, mark):
            half = lambda i, h: vt_ref[h * hd + r0:h * hd + r0 + nr,
                                       (Ks * NT + i) * T:(Ks * NT + i + 1) * T].astype(f32)
            i = job[0]
            ui = gate(half(i, 0), mark)
            if len(job) == 1:
                outs = [ui, half(i, 1) + LAM[i] * ui]
            else:
                j = job[1]
                mu = LAM[j] - LAM[i]
                su = _addsub(ui, half(j, 0), _sign(i, j))
                a2 = _addsub(half(i, 1), half(j, 1), _sign(i, j)) + LAM[i] * su
                a1 = a2 + (su if mu == 1 else su * mu)
                outs = [a1, a2, a1 - (ui if mu == 1 else ui * mu)]
            for k, x in enumerate(outs):
                vb_scr[Ks, BASE[b] + k, r0 // 2:(r0 + nr) // 2] = enc(x)

        return [(30, functools.partial(piece, r0), None) for r0 in range(0, hd, nr)]

    def offset(qi, m, ga):
        acc = []

        def piece(lo, mark):
            e = jnp.sum(jnp.exp2((ga[lo:lo + 2] - gate(m, mark)[None]) * (2 * c)), axis=0)
            acc[:] = [e + acc[0]] if acc else [e]

        def finish(mark):
            e = jnp.sum(gate(acc[0], mark), axis=0, keepdims=True)
            off = m + jnp.log2(e) * (0.5 / c)
            m_scr[0, :, qi * W:(qi + 1) * W] = jnp.broadcast_to(off, (8, W))

        return ([(20, functools.partial(piece, lo), qi) for lo in range(0, ga.shape[0], 2)]
                + [(30, finish, qi)])

    def combine(get, mark=None):
        diag = {job[0]: BASE[b] for b, job in enumerate(JOBS) if len(job) == 1}
        pairs = [(job, BASE[b]) for b, job in enumerate(JOBS) if len(job) == 2]
        x = [gate(get(diag[i]), mark) for i in range(NT)]
        for (i, j), b0 in pairs:
            mu = LAM[j] - LAM[i]
            g = get(b0) - get(b0 + 1) + get(b0 + 2)
            g = g if mu == 1 else g * (1.0 / mu)
            x[j], x[i] = x[j] + g, _addsub(x[i], g, _sign(i, j))
        y = [get(diag[i] + 1) for i in range(NT)]
        for (i, j), b0 in pairs:
            y[j], y[i] = y[j] + get(b0), _addsub(y[i], get(b0 + 1), _sign(i, j))
        y = [y[i] - LAM[i] * x[i] for i in range(NT)]
        return jnp.concatenate(x, axis=1), jnp.concatenate(y, axis=1)

    def post(Qs, ot_ref):
        cols = slice(Qs * NT * T, (Qs + 1) * NT * T)
        prev = []

        def piece(r0, mark):
            x, y = combine(lambda i: a_scr[Qs % 2, i, r0:r0 + 8], mark)
            x, y = x * l_scr[Qs % 2], y * l_scr[Qs % 2]
            if r0 % 16 == 0:
                prev[:] = [x, y]
                return
            ot_ref[r0 - 8:r0 + 8, cols] = jnp.concatenate([prev[0], x], axis=0).astype(bf16)
            ot_ref[hd + r0 - 8:hd + r0 + 8, cols] = jnp.concatenate([prev[1], y], axis=0).astype(bf16)

        return [(66, functools.partial(piece, r0), "post") for r0 in range(0, hd, 8)]

    class Phase1:
        def __init__(self, qt_ref, side):
            self.qt_ref, self.side, self.blocks = qt_ref, side, {}

        def begin(self, qi, m=None, gs=()):
            qt = self.qt_ref[:, qi * W:(qi + 1) * W]
            w = (qt[:2 * dc], qt[dc:], jnp.concatenate([qt[:dc], qt[2 * dc:]], axis=0))
            self.blocks[qi] = [w, m, list(gs)]

        def run(self, qi, ci):
            if qi not in self.blocks:
                self.begin(qi)
            st = self.blocks[qi]
            kl = [dec(k_scr[j, ci]) for j in range(3)]
            ts = [[None, None] for _ in range(3)]
            for h in range(2):
                for j in (2, 0, 1):
                    ts[j][h] = jnp.dot(kl[j], st[0][j][:, h * T:(h + 1) * T],
                                       preferred_element_type=f32)
            t1, t2, t3 = [jnp.concatenate(x, axis=1) for x in ts]
            s = jnp.concatenate([t1 + t3, t2 + t3], axis=0)
            s_scr[qi * nb + ci] = s
            gm = jnp.max(s.reshape(ng, GRP, 8, W), axis=1)
            mm = jnp.max(gm, axis=0)
            st[1] = mm if st[1] is None else jnp.maximum(st[1], mm)
            st[2].append(gm)
            if sum(x.shape[0] for x in st[2]) == nb * ng:
                m = jnp.max(st[1], axis=0, keepdims=True)
                self.side.extend(offset(qi, m, jnp.concatenate(st[2], axis=0)))
                del self.blocks[qi]
            return s

        def save(self):
            assert sorted(self.blocks) == list(range(nb - R, nb))
            for qi, st in self.blocks.items():
                m_scr[1, :, qi * W:(qi + 1) * W] = st[1]
                g_scr[qi - (nb - R)] = jnp.concatenate(st[2], axis=0)

    def start_group(h, slot):
        pltpu.make_async_copy(k_hbm.at[h], inbuf.at[slot, K], isem).start()
        pltpu.make_async_copy(q_hbm.at[h], inbuf.at[slot, Q], isem).start()
        pltpu.make_async_copy(v_hbm.at[h], inbuf.at[slot, V], isem).start()

    def wait_group(slot):
        pltpu.make_async_copy(inbuf.at[slot], inbuf.at[slot], isem).wait()

    def out_copy(h, slot):
        return pltpu.make_async_copy(obuf.at[slot], o_hbm.at[h], osem)

    def cols_copy(src, dst, lo, hi, i):
        return pltpu.make_async_copy(src.at[:, lo:hi], dst.at[:, lo:hi], psem.at[i])

    k0, q0, v0 = inbuf.at[2, K], inbuf.at[2, Q], inbuf.at[2, V]
    F = FIRST
    cps = [cols_copy(k_hbm.at[0], k0, 0, F, 0), cols_copy(q_hbm.at[0], q0, 0, F, 1),
           cols_copy(q_hbm.at[0], q0, F, 2 * F, 2), cols_copy(k_hbm.at[0], k0, F, 2 * F, 3),
           cols_copy(k_hbm.at[0], k0, 2 * F, S, 4), cols_copy(q_hbm.at[0], q0, 2 * F, S, 5),
           cols_copy(v_hbm.at[0], v0, 0, S, 6)]
    for d in cps:
        d.start()
    start_group(1, 0)
    a_scr[(ns - 1) % 2] = jnp.zeros(a_scr.shape[1:], f32)
    l_scr[...] = jnp.zeros(l_scr.shape, f32)
    side0 = []
    first = Phase1(q0, side0)
    done, prepped = set(tail_units), set()

    def rect(klo, khi, qlo, qhi):
        for qi in range(qlo // W, qhi // W):
            for ci in range(klo // W, khi // W):
                if (qi, ci) in done:
                    continue
                if ci not in prepped:
                    kprep(k0, ci)
                    prepped.add(ci)
                now = side0[:8]
                del side0[:8]
                s = first.run(qi, ci)
                done.add((qi, ci))
                for k, (_, f, _) in enumerate(now):
                    f(s[(k % 4) * 32 + (k // 4) * T:, (k // 4) * T:(k // 4 + 1) * T])

    cps[0].wait()
    for ci in range(F // W):
        kprep(k0, ci)
        prepped.add(ci)
    cps[1].wait()
    rect(0, F, 0, F)
    cps[2].wait()
    cps[3].wait()
    rect(0, F, F, 2 * F)
    rect(F, 2 * F, 0, F + W)
    for d in cps[4:]:
        d.wait()
    for Ks in range(ns):
        for b in range(len(JOBS)):
            side0.extend(vprep(v0, Ks, b))
    rect(F, 2 * F, F, 2 * F)
    rect(0, S, 0, S)
    for _, f, _ in side0:
        f(None)
    first.save()

    def step(g, slot, pslot, oslot, last, start_inputs, start_prev_out):
        ot_ref = obuf.at[oslot]
        side, outs, marks, prepped = [], [], [], set()
        tail = Phase1(inbuf.at[pslot, Q], side)
        for qi in range(nb - R, nb):
            tail.begin(qi, m_scr[1, :, qi * W:(qi + 1) * W], [g_scr[qi - (nb - R)]])
        start_inputs()
        side.extend(post(ns - 1, obuf.at[1 - oslot]))
        side.append((0, lambda mark: start_prev_out(), "post"))
        nxt = Phase1(inbuf.at[slot, Q], side)
        todo = [(tail, u) for u in tail_units]
        if not last:
            todo += [(nxt, u) for u in units[:-TAIL]]
        state = dict(budget=0, mark=0)

        def phase1():
            if todo:
                who, (qi, ci) = todo.pop(0)
                if who is nxt and ci not in prepped:
                    kprep(inbuf.at[slot, K], ci)
                    prepped.add(ci)
                who.run(qi, ci)

        def release(o):
            state["budget"] = min(state["budget"] + RATE, 2 * RATE + 40) if side else 0
            for mark in (o, o[hd // 2:]):
                if side and side[0][0] <= state["budget"]:
                    cost, f, _ = side.pop(0)
                    state["budget"] -= cost
                    f(mark)
                    while side and side[0][0] == 0:
                        side.pop(0)[1](None)

        def out_block(Qs):
            d = cols_copy(ot_ref, o_hbm.at[g], Qs * NT * T, (Qs + 1) * NT * T, Qs)
            d.start()
            outs.append(d)

        phase1()
        for Qs in range(ns):
            cols = slice(Qs * NT * T, (Qs + 1) * NT * T)
            assert not any(tag in range(Qs * R, (Qs + 1) * R) for _, _, tag in side)
            off, den, acc = m_scr[0, 0:1, cols], [None] * NT, {}
            final = last and Qs == ns - 1
            for Ks in range(ns):
                tiles = {}

                def prob(k, q):
                    if (k, q) not in tiles:
                        kt, qt = Ks * NT + k, Qs * NT + q
                        o = off[:, q * T:(q + 1) * T]
                        if Qs == ns - 1:
                            state["mark"] = max(state["mark"] + 1, len(marks) - (16 if last else 8))
                            o = gate(o, marks[state["mark"]])
                        s = s_scr[(qt // 2) * nb + kt // 2, (kt % 2) * T:(kt % 2 + 1) * T,
                                  (qt % 2) * T:(qt % 2 + 1) * T]
                        tiles[(k, q)] = jnp.exp2((s - o) * c)
                    return tiles[(k, q)]

                for b, job in enumerate(JOBS):
                    i = job[0]
                    if len(job) == 2:
                        j = job[1]
                        rhs = [prob(i, j), prob(j, i), prob(j, i) - prob(i, j)]
                    else:
                        rhs = []
                        for other in (lambda j: prob(i, j), lambda j: prob(j, i)):
                            plus, minus = prob(i, i), None
                            for j in range(NT):
                                if j != i and _sign(i, j) < 0:
                                    plus = plus + other(j)
                                elif j != i:
                                    minus = other(j) if minus is None else minus + other(j)
                            rhs.append(plus - minus)
                        tot, part = plus + minus, None
                        for r0 in range(T - 16, -1, -16):
                            x = tot[r0:r0 + 8] + tot[r0 + 8:r0 + 16]
                            part = x if part is None else part + x
                        den[i] = part if den[i] is None else den[i] + part
                    sw = ns if last else (b + Ks) % (ns - 1)
                    for k, x in enumerate(rhs):
                        p = BASE[b] + k
                        raw = vb_scr[Ks, p] if Qs <= sw else va_scr[Ks, p]
                        if Qs == sw:
                            va_scr[Ks, p] = raw
                        o = jnp.dot(dec(raw), x.astype(bf16), preferred_element_type=f32)
                        marks.append(o)
                        release(o)
                        if Ks == 0:
                            a_scr[Qs % 2, p] = o
                        elif Ks < ns - 1 or not final:
                            a_scr[Qs % 2, p] = a_scr[Qs % 2, p] + o
                        else:
                            acc[p] = a_scr[Qs % 2, p] + o
                        if ((p + 1) * TAIL) // NP > (p * TAIL) // NP and len(marks) > NP // TAIL + 1:
                            phase1()
                    if Qs == sw:
                        side.extend(vprep(inbuf.at[slot, V], Ks, b))
            assert not any(tag == "post" for _, _, tag in side)
            rl = 1.0 / jnp.sum(jnp.concatenate(den, axis=1), axis=0, keepdims=True)
            if final:
                ot_ref[:, cols] = (jnp.concatenate(combine(acc.get), axis=0) * rl).astype(bf16)
                out_block(Qs)
            else:
                l_scr[Qs % 2] = jnp.broadcast_to(rl, (8, NT * T))
                if Qs < ns - 1:
                    extra = [(0, lambda mark, Qs=Qs: out_block(Qs), "post")] if last else []
                    side[0:0] = post(Qs, ot_ref) + extra
        assert not todo and not side
        if not last:
            nxt.save()
        for d in outs:
            d.wait()

    def body(g, carry):
        slot, pslot, oslot = carry
        nslot = 3 - slot - pslot
        wait_group(slot)

        @pl.when(g >= 2)
        def _():
            out_copy(g - 2, oslot).wait()

        def start_inputs():
            @pl.when(g + 2 < N)
            def _():
                start_group(g + 2, nslot)

        def start_prev_out():
            @pl.when(g >= 1)
            def _():
                out_copy(g - 1, 1 - oslot).start()

        step(g, slot, pslot, oslot, False, start_inputs, start_prev_out)
        return nslot, slot, 1 - oslot

    lax.fori_loop(0, N - 1, body, (jnp.int32(0), jnp.int32(2), jnp.int32(0)))
    gl = N - 1
    out_copy(gl - 2, gl % 2).wait()
    step(gl, gl % 3, (gl - 1) % 3, gl % 2, True, lambda: None,
         lambda: out_copy(gl - 1, (gl - 1) % 2).start())
    out_copy(gl - 1, (gl - 1) % 2).wait()


@jax.jit
def pallas_standalone__mha_softmax__prompt_kernel(q: jax.Array, k: jax.Array, v: jax.Array):
    B, H, S, D = q.shape
    N = B * H
    assert k.shape == q.shape and v.shape == q.shape
    assert D == 192 and S == 2048 and N >= 3
    nb, ns = S // W, S // (NT * T)
    tr = lambda x: jnp.swapaxes(x, 2, 3).reshape(N, D, S)
    hbm = pl.BlockSpec(memory_space=pl.ANY)
    ot = pl.pallas_call(
        _kernel,
        in_specs=[hbm] * 3,
        out_specs=hbm,
        out_shape=jax.ShapeDtypeStruct((N, D, S), q.dtype),
        scratch_shapes=[
            pltpu.VMEM((3, 3, D, S), bf16),
            pltpu.VMEM((2, D, S), bf16),
            pltpu.VMEM((3, nb, T // 2, T), u32),
            pltpu.VMEM((2, 8, S), f32),
            pltpu.VMEM((R, (nb - TAIL // R) * (W // (8 * GRP)), 8, W), f32),
            pltpu.VMEM((nb * nb, W, W), f32),
            pltpu.VMEM((2, NP, D // 2, T), f32),
            pltpu.VMEM((2, 8, NT * T), f32),
            pltpu.VMEM((ns, NP, D // 4, T), u32),
            pltpu.VMEM((ns, NP, D // 4, T), u32),
            pltpu.SemaphoreType.DMA(()),
            pltpu.SemaphoreType.DMA(()),
            pltpu.SemaphoreType.DMA((7,)),
        ],
        compiler_params=pltpu.CompilerParams(
            vmem_limit_bytes=100 * 1024 * 1024,
            disable_bounds_checks=True,
        ),
        name="mha",
    )(tr(q), tr(k), tr(v))
    return jnp.swapaxes(ot.reshape(B, H, D, S), 2, 3)
```

```python
import functools
import math

import numpy as np
import jax
import jax.numpy as jnp
from jax import lax
import jax.experimental.pallas as pl
import jax.experimental.pallas.tpu as pltpu

f32 = jnp.float32
bf16 = jnp.bfloat16

T = 128
W = 2 * T
NT = 4
R = NT * T // W
LAM = (-1.375, -0.375, 0.375, 1.375)
NEG = ((0, 3), (1, 2))
JOBS = ((2, 3), (0, 3), (1, 3), (3,), (0, 2), (1, 2), (2,), (0, 1), (1,), (0,))
BASE = [int(x) for x in np.cumsum([0] + [len(j) + 1 for j in JOBS])]
NP = BASE[-1]
GRP = 16
TAIL = R * R
FIRST = 512
P1POS = (5, 11, 18, 24)
RATE = 33
CAP = 108
VCOST = 34
PCOST = 66
MARK2 = 32
OG = 2
DLAG = 9
ELAG = 15
PSIDE = 8
SW = (0, 1)
PV0 = 2
V, K, Q = 0, 1, 2


def _sign(i, j):
    return -1 if (min(i, j), max(i, j)) in NEG else 1


def _addsub(x, y, s):
    return x + y if s > 0 else x - y


def _kernel(q_hbm, k_hbm, v_hbm, o_hbm, inbuf, obuf, k_scr, m_scr, g_scr, s_scr, a_scr, l_scr,
            v_scr, isem, osem, psem):
    N, D, S = q_hbm.shape
    nb, ns, hd, dc, ng = S // W, S // (NT * T), D // 2, D // 3, W // (8 * GRP)
    c = float(np.asarray(D ** -0.5, dtype=bf16)) * math.log2(math.e)
    units = [(Qs * R + a, Ks * R + b) for Qs in range(ns) for Ks in range(ns)
             for a in range(R) for b in range(R)]
    tail_units = units[-TAIL:]

    never = lax.fori_loop(0, 2, lambda i, x: 1 - x, jnp.int32(0)) < 0

    def gate(x, mark):
        if mark is None:
            return x
        return jnp.where(never, jnp.tile(mark[:x.shape[0]], (1, x.shape[1] // T)), x)

    def kprep(kt_ref, ci):
        kt = kt_ref[:, ci * W:(ci + 1) * W]
        a = kt[:, :T].astype(f32)
        b = kt[:, T:].astype(f32)
        l1 = jnp.concatenate([a[:dc] - b[:dc], a[dc:2 * dc]], axis=0)
        l2 = jnp.concatenate([b[dc:2 * dc], b[2 * dc:] - a[2 * dc:]], axis=0)
        l3 = jnp.concatenate([b[:dc], a[2 * dc:]], axis=0)
        kl = [x.T.astype(bf16) for x in (l1, l2, l3)]
        if ci >= nb - R:
            for j, x in enumerate(kl):
                k_scr[j, ci - (nb - R)] = x
        return kl

    def vprep(vt_ref, Ks, b):
        job = JOBS[b]
        nr = 16 if len(job) == 2 else 32

        def piece(r0, mark):
            half = lambda i, h: vt_ref[h * hd + r0:h * hd + r0 + nr,
                                       (Ks * NT + i) * T:(Ks * NT + i + 1) * T].astype(f32)
            i = job[0]
            ui = gate(half(i, 0), mark)
            if len(job) == 1:
                outs = [ui, half(i, 1) + LAM[i] * ui]
            else:
                j = job[1]
                mu = LAM[j] - LAM[i]
                s, uj = _sign(i, j), half(j, 0)
                a3 = _addsub(half(i, 1) + LAM[i] * ui, half(j, 1) + LAM[j] * uj, s)
                a3 = a3.astype(bf16).astype(f32)
                outs = [a3 + (ui if mu == 1 else ui * mu),
                        _addsub(a3, uj if mu == 1 else uj * mu, -s), a3]
            for k, x in enumerate(outs):
                v_scr[Ks, BASE[b] + k, r0:r0 + nr] = x.astype(bf16)

        return [(VCOST, functools.partial(piece, r0), None) for r0 in range(0, hd, nr)]

    def offset(qi, m, ga):
        acc = []

        def piece(lo, mark):
            e = jnp.sum(jnp.exp2((ga[lo:lo + OG] - gate(m, mark)[None]) * (2 * c)), axis=0)
            acc[:] = [e + acc[0]] if acc else [e]

        def finish(mark):
            e = jnp.sum(gate(acc[0], mark), axis=0, keepdims=True)
            off = m + jnp.log2(e) * (0.75 / c)
            m_scr[0, :, qi * W:(qi + 1) * W] = jnp.broadcast_to(off, (8, W))

        return ([(4 + 8 * OG, functools.partial(piece, lo), qi) for lo in range(0, ga.shape[0], OG)]
                + [(30, finish, qi)])

    def combine(get, mark=None):
        diag = {job[0]: BASE[b] for b, job in enumerate(JOBS) if len(job) == 1}
        pairs = [(job, BASE[b]) for b, job in enumerate(JOBS) if len(job) == 2]
        x = [gate(get(diag[i]), mark) for i in range(NT)]
        for (i, j), b0 in pairs:
            mu = LAM[j] - LAM[i]
            g = get(b0) - get(b0 + 1) + get(b0 + 2)
            g = g if mu == 1 else g * (1.0 / mu)
            x[j], x[i] = x[j] + g, _addsub(x[i], g, _sign(i, j))
        y = [get(diag[i] + 1) for i in range(NT)]
        for (i, j), b0 in pairs:
            y[j], y[i] = y[j] + get(b0), _addsub(y[i], get(b0 + 1), _sign(i, j))
        y = [y[i] - LAM[i] * x[i] for i in range(NT)]
        return jnp.concatenate(x, axis=1), jnp.concatenate(y, axis=1)

    def post(Qs, ot_ref):
        cols = slice(Qs * NT * T, (Qs + 1) * NT * T)
        prev = []

        def piece(r0, mark):
            prods, rl = a_scr[Qs % 2, :, r0:r0 + 8, :], l_scr[Qs % 2]
            x, y = combine([prods[i] for i in range(NP)].__getitem__, mark)
            x, y = x * rl, y * rl
            if r0 % 16 == 0:
                prev[:] = [x, y]
                return
            ot_ref[r0 - 8:r0 + 8, cols] = jnp.concatenate([prev[0], x], axis=0).astype(bf16)
            ot_ref[hd + r0 - 8:hd + r0 + 8, cols] = jnp.concatenate([prev[1], y], axis=0).astype(bf16)

        return [(PCOST, functools.partial(piece, r0), "post") for r0 in range(0, hd, 8)]

    class Phase1:
        def __init__(self, qt_ref, side, left):
            self.qt_ref, self.side, self.left = qt_ref, side, left
            self.blocks, self.kl = {}, {}

        def begin(self, qi, m=None, gs=()):
            qt = self.qt_ref[:, qi * W:(qi + 1) * W]
            w = (qt[:2 * dc], qt[dc:], jnp.concatenate([qt[:dc], qt[2 * dc:]], axis=0))
            self.blocks[qi] = [w, m, list(gs)]

        def run(self, qi, ci):
            if qi not in self.blocks:
                self.begin(qi)
            st = self.blocks[qi]
            if ci not in self.kl:
                self.kl[ci] = self.left(ci)
            kl = self.kl[ci]
            ts = [[None, None] for _ in range(3)]
            for h in range(2):
                for j in (2, 0, 1):
                    ts[j][h] = jnp.dot(kl[j], st[0][j][:, h * T:(h + 1) * T],
                                       preferred_element_type=f32)
            t1, t2, t3 = [jnp.concatenate(x, axis=1) for x in ts]
            s = jnp.concatenate([t1 + t3, t2 + t3], axis=0)
            s_scr[qi * nb + ci] = s
            gm = jnp.max(s.reshape(ng, GRP, 8, W), axis=1)
            mm = jnp.max(gm, axis=0)
            st[1] = mm if st[1] is None else jnp.maximum(st[1], mm)
            st[2].append(gm)
            if sum(x.shape[0] for x in st[2]) == nb * ng:
                m = jnp.max(st[1], axis=0, keepdims=True)
                self.side.extend(offset(qi, m, jnp.concatenate(st[2], axis=0)))
                del self.blocks[qi]
            return s

        def save(self):
            assert sorted(self.blocks) == list(range(nb - R, nb))
            for qi, st in self.blocks.items():
                m_scr[1, :, qi * W:(qi + 1) * W] = st[1]
                g_scr[qi - (nb - R)] = jnp.concatenate(st[2], axis=0)

    def start_group(h, slot):
        pltpu.make_async_copy(k_hbm.at[h], inbuf.at[slot, K], isem).start()
        pltpu.make_async_copy(q_hbm.at[h], inbuf.at[slot, Q], isem).start()
        pltpu.make_async_copy(v_hbm.at[h], inbuf.at[slot, V], isem).start()

    def wait_group(slot):
        pltpu.make_async_copy(inbuf.at[slot], inbuf.at[slot], isem).wait()

    def out_copy(h, slot):
        return pltpu.make_async_copy(obuf.at[slot], o_hbm.at[h], osem)

    def cols_copy(src, dst, lo, hi, i):
        return pltpu.make_async_copy(src.at[:, lo:hi], dst.at[:, lo:hi], psem.at[i])

    k0, q0, v0 = inbuf.at[2, K], inbuf.at[2, Q], inbuf.at[2, V]
    F = FIRST
    cps = [cols_copy(k_hbm.at[0], k0, 0, F, 0), cols_copy(q_hbm.at[0], q0, 0, F, 1),
           cols_copy(q_hbm.at[0], q0, F, 2 * F, 2), cols_copy(k_hbm.at[0], k0, F, 2 * F, 3),
           cols_copy(k_hbm.at[0], k0, 2 * F, S, 4), cols_copy(q_hbm.at[0], q0, 2 * F, S, 5),
           cols_copy(v_hbm.at[0], v0, 0, S, 6)]
    for d in cps:
        d.start()
    start_group(1, 0)
    a_scr[(ns - 1) % 2] = jnp.zeros(a_scr.shape[1:], f32)
    l_scr[...] = jnp.zeros(l_scr.shape, f32)
    side0 = []
    first = Phase1(q0, side0, functools.partial(kprep, k0))
    done = set(tail_units)

    def rect(klo, khi, qlo, qhi):
        for qi in range(qlo // W, qhi // W):
            for ci in range(klo // W, khi // W):
                if (qi, ci) in done:
                    continue
                now = side0[:PSIDE]
                del side0[:PSIDE]
                s = first.run(qi, ci)
                done.add((qi, ci))
                for k, (_, f, _) in enumerate(now):
                    h, r0 = divmod(k * W // PSIDE // 8 * 8, T)
                    f(s[min(r0, T - 32) + h * T:, h * T:(h + 1) * T])

    cps[0].wait()
    for ci in range(F // W):
        first.kl[ci] = kprep(k0, ci)
    cps[1].wait()
    rect(0, F, 0, F)
    cps[2].wait()
    cps[3].wait()
    rect(0, F, F, 2 * F)
    rect(F, 2 * F, 0, F)
    cps[4].wait()
    cps[5].wait()
    rect(F, 2 * F, F, 2 * F)
    rect(0, S, 0, PV0 * W)
    cps[6].wait()
    for Ks in range(ns):
        for b in range(len(JOBS)):
            side0.extend(vprep(v0, Ks, b))
    rect(0, S, 0, S)
    for _, f, _ in side0:
        f(None)
    first.save()

    def step(g, slot, pslot, oslot, last, start_inputs, start_prev_out):
        ot_ref = obuf.at[oslot]
        side, outs, marks, lhs = [], [], [], {}
        tail = Phase1(inbuf.at[pslot, Q], side,
                      lambda ci: [k_scr[j, ci - (nb - R)] for j in range(3)])
        for qi in range(nb - R, nb):
            tail.begin(qi, m_scr[1, :, qi * W:(qi + 1) * W], [g_scr[qi - (nb - R)]])
        start_inputs()
        side.extend(post(ns - 1, obuf.at[1 - oslot]))
        side.append((0, lambda mark: start_prev_out(), "post"))
        nxt = Phase1(inbuf.at[slot, Q], side, functools.partial(kprep, inbuf.at[slot, K]))
        todo = [(tail, u) for u in tail_units]
        if not last:
            todo += [(nxt, u) for u in units[:-TAIL]]
        state = dict(budget=0, mark=0)

        def phase1():
            if todo:
                who, (qi, ci) = todo.pop(0)
                who.run(qi, ci)

        def release(o):
            state["budget"] = min(state["budget"] + RATE, CAP) if side else 0
            for mark in (o, o[MARK2:]):
                if side and side[0][0] <= state["budget"]:
                    cost, f, _ = side.pop(0)
                    state["budget"] -= cost
                    f(mark)
                    while side and side[0][0] == 0:
                        side.pop(0)[1](None)

        def out_block(Qs):
            d = cols_copy(ot_ref, o_hbm.at[g], Qs * NT * T, (Qs + 1) * NT * T, Qs)
            d.start()
            outs.append(d)

        phase1()
        for Qs in range(ns):
            cols = slice(Qs * NT * T, (Qs + 1) * NT * T)
            assert not any(tag in range(Qs * R, (Qs + 1) * R) for _, _, tag in side)
            off, den, acc = m_scr[0, 0:1, cols], [None] * NT, {}
            final = last and Qs == ns - 1
            for Ks in range(ns):
                tiles = {}

                def prob(k, q):
                    if (k, q) not in tiles:
                        kt, qt = Ks * NT + k, Qs * NT + q
                        o = off[:, q * T:(q + 1) * T]
                        if Qs == ns - 1:
                            state["mark"] = max(state["mark"] + 1, len(marks) - (ELAG if last else DLAG))
                            o = gate(o, marks[state["mark"]])
                        s = s_scr[(qt // 2) * nb + kt // 2, (kt % 2) * T:(kt % 2 + 1) * T,
                                  (qt % 2) * T:(qt % 2 + 1) * T]
                        tiles[(k, q)] = jnp.exp2((s - o) * c)
                    return tiles[(k, q)]

                for b, job in enumerate(JOBS):
                    i = job[0]
                    if len(job) == 2:
                        j = job[1]
                        rhs = [prob(i, j), prob(j, i), prob(j, i) - prob(i, j)]
                    else:
                        rhs = []
                        for other in (lambda j: prob(i, j), lambda j: prob(j, i)):
                            plus, minus = prob(i, i), None
                            for j in range(NT):
                                if j != i and _sign(i, j) < 0:
                                    plus = plus + other(j)
                                elif j != i:
                                    minus = other(j) if minus is None else minus + other(j)
                            rhs.append(plus - minus)
                        tot, part = plus + minus, None
                        for r0 in range(T - 16, -1, -16):
                            x = tot[r0:r0 + 8] + tot[r0 + 8:r0 + 16]
                            part = x if part is None else part + x
                        den[i] = part if den[i] is None else den[i] + part
                    sw = SW[b % len(SW)]
                    for k, x in enumerate(rhs):
                        p = BASE[b] + k
                        if Qs <= sw:
                            lhs[Ks, p] = v_scr[Ks, p]
                        o = jnp.dot(lhs[Ks, p], x.astype(bf16), preferred_element_type=f32)
                        marks.append(o)
                        release(o)
                        if Ks == 0:
                            a_scr[Qs % 2, p] = o
                        elif Ks < ns - 1 or not final:
                            a_scr[Qs % 2, p] = a_scr[Qs % 2, p] + o
                        else:
                            acc[p] = a_scr[Qs % 2, p] + o
                        if p in P1POS and len(marks) > P1POS[0] + 1:
                            phase1()
                    if Qs == sw and not last:
                        side.extend(vprep(inbuf.at[slot, V], Ks, b))
            assert not any(tag == "post" for _, _, tag in side)
            rl = 1.0 / jnp.sum(jnp.concatenate(den, axis=1), axis=0, keepdims=True)
            if final:
                ot_ref[:, cols] = (jnp.concatenate(combine(acc.get), axis=0) * rl).astype(bf16)
                out_block(Qs)
            else:
                l_scr[Qs % 2] = jnp.broadcast_to(rl, (8, NT * T))
                if Qs < ns - 1:
                    extra = [(0, lambda mark, Qs=Qs: out_block(Qs), "post")] if last else []
                    side[0:0] = post(Qs, ot_ref) + extra
        assert not todo and not side
        if not last:
            nxt.save()
        for d in outs:
            d.wait()

    def body(g, carry):
        slot, pslot, oslot = carry
        nslot = 3 - slot - pslot
        wait_group(slot)

        @pl.when(g >= 2)
        def _():
            out_copy(g - 2, oslot).wait()

        def start_inputs():
            @pl.when(g + 2 < N)
            def _():
                start_group(g + 2, nslot)

        def start_prev_out():
            @pl.when(g >= 1)
            def _():
                out_copy(g - 1, 1 - oslot).start()

        step(g, slot, pslot, oslot, False, start_inputs, start_prev_out)
        return nslot, slot, 1 - oslot

    lax.fori_loop(0, N - 1, body, (jnp.int32(0), jnp.int32(2), jnp.int32(0)))
    gl = N - 1
    out_copy(gl - 2, gl % 2).wait()
    step(gl, gl % 3, (gl - 1) % 3, gl % 2, True, lambda: None,
         lambda: out_copy(gl - 1, (gl - 1) % 2).start())
    out_copy(gl - 1, (gl - 1) % 2).wait()


@jax.jit
def pallas_standalone__mha_softmax__prompt_kernel(q: jax.Array, k: jax.Array, v: jax.Array):
    B, H, S, D = q.shape
    N = B * H
    assert k.shape == q.shape and v.shape == q.shape
    assert D == 192 and S == 2048 and N >= 3
    nb, ns = S // W, S // (NT * T)
    tr = lambda x: jnp.swapaxes(x, 2, 3).reshape(N, D, S)
    hbm = pl.BlockSpec(memory_space=pl.ANY)
    ot = pl.pallas_call(
        _kernel,
        in_specs=[hbm] * 3,
        out_specs=hbm,
        out_shape=jax.ShapeDtypeStruct((N, D, S), q.dtype),
        scratch_shapes=[
            pltpu.VMEM((3, 3, D, S), bf16),
            pltpu.VMEM((2, D, S), bf16),
            pltpu.VMEM((3, R, T, T), bf16),
            pltpu.VMEM((2, 8, S), f32),
            pltpu.VMEM((R, (nb - TAIL // R) * (W // (8 * GRP)), 8, W), f32),
            pltpu.VMEM((nb * nb, W, W), f32),
            pltpu.VMEM((2, NP, D // 2, T), f32),
            pltpu.VMEM((2, 8, NT * T), f32),
            pltpu.VMEM((ns, NP, D // 2, T), bf16),
            pltpu.SemaphoreType.DMA(()),
            pltpu.SemaphoreType.DMA(()),
            pltpu.SemaphoreType.DMA((7,)),
        ],
        compiler_params=pltpu.CompilerParams(
            vmem_limit_bytes=100 * 1024 * 1024,
            disable_bounds_checks=True,
        ),
        name="mha",
    )(tr(q), tr(k), tr(v))
    return jnp.swapaxes(ot.reshape(B, H, D, S), 2, 3)
```
